```python
import jax
import jax.numpy as jnp

def _softmax(x, axis=-1):
    return jax.nn.softmax(x, axis=axis)
def _gelu(x):
    return jax.nn.gelu(x, approximate=True)
def _silu(x):
    return jax.nn.silu(x)
def _sigmoid(x):
    return jax.nn.sigmoid(x)
def _layernorm(x, axis=-1, eps=1e-5):
    m = jnp.mean(x, axis=axis, keepdims=True)
    v = jnp.var(x, axis=axis, keepdims=True)
    return (x - m) / jnp.sqrt(v + eps)
def _scatter_add(tgt, idx, src, axis=0):
    return tgt.at[idx].add(src)
def _segment_sum(src, seg, n):
    return jax.ops.segment_sum(src, seg, n)
class _Rng:
    def __init__(self, key):
        self._k = key
    def _next(self):
        self._k, sub = jax.random.split(self._k)
        return sub
    def normal(self, shape):
        return jax.random.normal(self._next(), shape, dtype=jnp.bfloat16)
    def randint(self, lo, hi, shape):
        return jax.random.randint(self._next(), shape, lo, hi, dtype=jnp.int32)
    def uniform(self, shape, lo=0.0, hi=1.0):
        return jax.random.uniform(self._next(), shape, jnp.bfloat16, lo, hi)
    def permutation(self, n):
        return jax.random.permutation(self._next(), n)


kernel_name = 'recurrent_scan__sliding_block_cached__mixer_s_mlp__decode'

def _fwd_setup_inputs():
    _rng = _Rng(jax.random.key(int.from_bytes(__import__("os").urandom(4), "little")))
    _w = (lambda a: (lambda t: t.astype(jnp.bfloat16) if jnp.issubdtype(t.dtype, jnp.floating) else t)(jnp.asarray(a)))
    def _A_setup():
        B, Sq, D = 4, 1, 512
        Hq, Hkv, Sk, Dh = 32, 8, 8192, 128
        assert Hq % Hkv == 0, (Hq, Hkv)
        return {
            "x": _w((lambda *s: _rng.normal(s) * 0.05)(B, Sq, D)),
            "k_cache": _w((lambda *s: _rng.normal(s) * 0.05)(B, Hkv, Sk, Dh)),
            "v_cache": _w((lambda *s: _rng.normal(s) * 0.05)(B, Hkv, Sk, Dh)),
            "wq": _w((lambda *s: _rng.normal(s) * 0.05)(D, Hq * Dh) * (D ** -0.5)),
            "wo": _w((lambda *s: _rng.normal(s) * 0.05)(Hq * Dh, D) * ((Hq * Dh) ** -0.5)),
        }
    _A_in = _A_setup()

    def _B_setup():
        B, S, D, F = 4, 1, 512, 1792
        return {
            "x":  _w((lambda *s: _rng.normal(s) * 0.05)(B, S, D)),
            "w1": _w((lambda *s: _rng.normal(s) * 0.05)(D, D) * (D ** -0.5)),
            "w2": _w((lambda *s: _rng.normal(s) * 0.05)(D, D) * (D ** -0.5)),
            "w3": _w((lambda *s: _rng.normal(s) * 0.05)(D, F) * (D ** -0.5)),
            "w4": _w((lambda *s: _rng.normal(s) * 0.05)(F, D) * (F ** -0.5)),
        }
    _B_in = _B_setup()

    return {
        "A_x": _A_in["x"],
        "A_k_cache": _A_in["k_cache"],
        "A_v_cache": _A_in["v_cache"],
        "A_wq": _A_in["wq"],
        "A_wo": _A_in["wo"],
        "B_x": _B_in["x"],
        "B_w1": _B_in["w1"],
        "B_w2": _B_in["w2"],
        "B_w3": _B_in["w3"],
        "B_w4": _B_in["w4"],
    }

def _fwd_reference(A_x, A_k_cache, A_v_cache, A_wq, A_wo, B_x, B_w1, B_w2, B_w3, B_w4):
    def _A_ref(x, k_cache, v_cache, wq, wo):
        B, Sq, D = x.shape
        Hq, Dh = 32, 128
        Hkv, Sk = k_cache.shape[1], k_cache.shape[2]
        W = min(4096, max(256, Sk // 4))
        rep = Hq // Hkv
        q = (lambda x, *d: x.transpose(*d))((x @ wq).reshape(B, Sq, Hq, Dh), 0, 2, 1, 3)
        k = jnp.repeat(k_cache[:, :, Sk - W:, :], rep, axis=1)
        v = jnp.repeat(v_cache[:, :, Sk - W:, :], rep, axis=1)
        scores = jnp.einsum("bhqd,bhkd->bhqk", q, k) * (Dh ** -0.5)
        p = _softmax(scores, axis=-1)
        o = jnp.einsum("bhqk,bhkd->bhqd", p, v)
        return (lambda x, *d: x.transpose(*d))(o, 0, 2, 1, 3).reshape(B, Sq, Hq * Dh) @ wo

    def _B_ref(x, w1, w2, w3, w4):
        B, S, D = x.shape
        h = _gelu(_layernorm(x, axis=-1) @ w1)
        c = D // 4
        g0 = jnp.pad(h[:, :, 0*c:1*c], ((0, 0), (1, 0), (0, 0)))[:, :S, :]
        g1 = jnp.pad(h[:, :, 1*c:2*c], ((0, 0), (0, 1), (0, 0)))[:, 1:, :]
        g2 = jnp.pad(h[:, :, 2*c:3*c], ((0, 0), (2, 0), (0, 0)))[:, :S, :]
        g3 = jnp.pad(h[:, :, 3*c:   ], ((0, 0), (0, 2), (0, 0)))[:, 2:, :]
        hs = jnp.concatenate([g0, g1, g2, g3], axis=-1) @ w2
        x1 = x + hs
        h2 = _gelu(_layernorm(x1, axis=-1) @ w3) @ w4
        return x1 + h2

    x = A_x
    xn = _layernorm(x, axis=-1)
    s = _A_ref(xn, A_k_cache, A_v_cache, A_wq, A_wo)
    g = _silu(_B_ref(xn, B_w1, B_w2, B_w3, B_w4))
    return x + s * g


def setup_inputs():
    _inp = _fwd_setup_inputs()
    _gk = jax.random.fold_in(jax.random.key(int.from_bytes(__import__("os").urandom(4), "little")), 2**31 - 1)
    _shapes = [[4, 1, 512]]
    _dtypes = ['bfloat16']
    _gks = jax.random.split(_gk, len(_shapes))
    _gs = [jax.random.normal(k, s, dtype=jnp.dtype(d)) * 0.05 for k, s, d in zip(_gks, _shapes, _dtypes)]
    _inp["grad_out"] = _gs[0]
    return _inp

def reference(A_x, A_k_cache, A_v_cache, A_wq, A_wo, B_w3, B_w4, B_x, B_w1, B_w2, grad_out):
    _const = dict(B_x=B_x, B_w1=B_w1, B_w2=B_w2)
    def _f(*_d):
        return _fwd_reference(**{'A_x': _d[0], 'A_k_cache': _d[1], 'A_v_cache': _d[2], 'A_wq': _d[3], 'A_wo': _d[4], 'B_w3': _d[5], 'B_w4': _d[6], **_const})
    _out, _vjp = jax.vjp(_f, A_x, A_k_cache, A_v_cache, A_wq, A_wo, B_w3, B_w4)
    _grads = _vjp(grad_out)
    _out0 = jnp.asarray(_out)
    return (_out0, *[jnp.asarray(_g) for _g in _grads])
```

```python
import jax
import jax.numpy as jnp
from jax import lax
import jax.experimental.pallas as pl
import jax.experimental.pallas.tpu as pltpu

F32 = jnp.float32
BF16 = jnp.bfloat16

HQ = 32
DH = 128
EPS = 1e-5

STREAMS = 8
MLP_STREAMS = 4
READ_ROWS = 16
READ_COLS = 256
WRITE_ROWS = 112

NN = (((1,), (0,)), ((), ()))
NT = (((1,), (1,)), ((), ()))
TN = (((0,), (0,)), ((), ()))


def _dot(a, b, dims):
    return lax.dot_general(
        a.astype(BF16), b.astype(BF16), dims, preferred_element_type=F32
    )


def _layernorm(x):
    xc = x - jnp.mean(x, axis=-1, keepdims=True)
    var = jnp.mean(xc * xc, axis=-1, keepdims=True)
    rstd = 1.0 / jnp.sqrt(var + EPS)
    return xc * rstd, rstd


def _layernorm_bwd(dy, y, rstd):
    return rstd * (
        dy
        - jnp.mean(dy, axis=-1, keepdims=True)
        - y * jnp.mean(dy * y, axis=-1, keepdims=True)
    )


def _gelu_and_grad(z):
    c0, c1 = 0.7978845608028654, 0.044715
    t = jnp.tanh(c0 * (z + c1 * z * z * z))
    cdf = 0.5 * (1.0 + t)
    dcdf = 0.5 * (1.0 - t * t) * c0 * (1.0 + 3.0 * c1 * z * z)
    return z * cdf, cdf + z * dcdf


def _copy(src, dst, sem, priority=0):
    pltpu.make_async_copy(src, dst, sem).start(priority=priority)


def _wait(ref, sem):
    pltpu.make_async_copy(ref, ref, sem).wait()


def _loop(lo, hi, body):
    def step(i, carry):
        body(i)
        return carry

    lax.fori_loop(lo, hi, step, None)


def _ds(start, size, multiple):
    if isinstance(start, int):
        return pl.ds(start, size)
    return pl.ds(pl.multiple_of(start, multiple), size)


def _matrix(ref):
    streams, n_rows, n_cols = ref.shape
    return ref[...].reshape(streams * n_rows, n_cols)


def _kernel(
    x_h, go_h, k_h, v_h, wq_h, wo_h, w3_h, w4_h,
    out_h, dx_h, dk_h, dv_h, dwq_h, dwo_h, dw3_h, dw4_h,
    x_v, go_v, k_v, v_v, wq_v, wo_v, w3_v, w4_v,
    out_v, dx_v, dk_v, dv_v, dwq_v, dwo_v, dw3_v, dw4_v,
    zero_v, q_s, do_s, o_s, dq_s,
    sems,
):
    n_pair, cache_len, _ = k_h.shape
    n_group = dk_h.shape[1]
    win = k_v.shape[1]
    front = cache_len - win
    batch = x_h.shape[0]
    rep = batch * HQ // n_pair
    scale = DH**-0.5
    (s_x, s_go, s_k, s_v, s_wq, s_wo, s_w3, s_w4, s_zk, s_zv,
     s_out, s_dx, s_dk, s_dv, s_dwq, s_dwo, s_dw3, s_dw4) = (
        sems.at[i] for i in range(18))

    def read_group(g):
        pairs = pl.ds(g * STREAMS, STREAMS)

        def read_rows(i):
            src = _ds(front + i * READ_ROWS, READ_ROWS, READ_ROWS)
            dst = _ds(i * READ_ROWS, READ_ROWS, READ_ROWS)
            _copy(k_h.at[pairs, src, :], k_v.at[pairs, dst, :], s_k, 0)
            _copy(v_h.at[pairs, src, :], v_v.at[pairs, dst, :], s_v, 1)

        _loop(0, win // READ_ROWS, read_rows)

    _loop(0, n_pair // STREAMS, read_group)

    _copy(x_h, x_v, s_x, 0)
    _copy(go_h, go_v, s_go, 1)

    def read_weights(wide_h, wide_v, wide_sem, tall_h, tall_v, tall_sem):
        per_wide = wide_h.shape[2] // READ_COLS
        per_tall = tall_h.shape[2] // READ_COLS

        def read_rows(i):
            for c in range(per_wide):
                tile = (slice(None), _ds(i * 8, 8, 8),
                        pl.ds(c * READ_COLS, READ_COLS))
                _copy(wide_h.at[tile], wide_v.at[tile], wide_sem, 0)
                j = i * per_wide + c
                tile = (slice(None), _ds(lax.div(j, per_tall) * 8, 8, 8),
                        _ds(lax.rem(j, per_tall) * READ_COLS, READ_COLS, READ_COLS))
                _copy(tall_h.at[tile], tall_v.at[tile], tall_sem, 1)

        _loop(0, wide_h.shape[1] // 8, read_rows)

    read_weights(wq_h, wq_v, s_wq, wo_h, wo_v, s_wo)
    read_weights(w3_h, w3_v, s_w3, w4_h, w4_v, s_w4)

    zero_v[...] = jnp.zeros(zero_v.shape, BF16)
    n_zero, zero_tail = divmod(front, WRITE_ROWS)
    n_win, win_tail = divmod(win, WRITE_ROWS)

    def write_zeros(dst_h, sem, g, lo=0, hi=n_zero):
        def body(i):
            dst = _ds(i * WRITE_ROWS, WRITE_ROWS, 16)
            _copy(zero_v, dst_h.at[:, g, dst, :], sem)

        _loop(lo, hi, body)
        if hi == n_zero and zero_tail:
            _copy(zero_v.at[:, pl.ds(0, zero_tail), :],
                  dst_h.at[:, g, pl.ds(front - zero_tail, zero_tail), :], sem)

    def write_window(src_v, dst_h, sem, g):
        def body(i):
            src = _ds(i * WRITE_ROWS, WRITE_ROWS, 16)
            dst = _ds(front + i * WRITE_ROWS, WRITE_ROWS, 16)
            _copy(src_v.at[:, g, src, :], dst_h.at[:, g, dst, :], sem)

        _loop(0, n_win, body)
        if win_tail:
            _copy(src_v.at[:, g, pl.ds(win - win_tail, win_tail), :],
                  dst_h.at[:, g, pl.ds(cache_len - win_tail, win_tail), :], sem)

    def write_rows(src_v, dst_h, sem, i, n_rows, cols=slice(None)):
        tile = (slice(None), _ds(i * n_rows, n_rows, n_rows), cols)
        _copy(src_v.at[tile], dst_h.at[tile], sem)

    def store(ref, value):
        ref[...] = value.astype(BF16).reshape(ref.shape)

    write_zeros(dk_h, s_zk, 0)
    for ref, sem in ((x_v, s_x), (go_v, s_go), (w3_v, s_w3), (w4_v, s_w4),
                     (wq_v, s_wq), (wo_v, s_wo), (k_v, s_k), (v_v, s_v)):
        _wait(ref, sem)
    x = x_v[...].astype(F32)
    go = go_v[...].astype(F32)
    xn, rstd1 = _layernorm(x)
    ln2, rstd2 = _layernorm(xn)
    act, dact = _gelu_and_grad(_dot(ln2, _matrix(w3_v), NN))
    y = xn + _dot(act, _matrix(w4_v), NN)
    sig = jax.nn.sigmoid(y)
    gate = y * sig
    d_s = go * gate
    q = _dot(xn, _matrix(wq_v), NN)
    d_o = _dot(d_s, _matrix(wo_v), NT)
    for h in range(HQ):
        q_s[pl.ds(h, batch, stride=HQ), :] = q[:, h * DH:(h + 1) * DH]
        do_s[pl.ds(h, batch, stride=HQ), :] = d_o[:, h * DH:(h + 1) * DH]
    _loop(1, n_group, lambda g: write_zeros(dk_h, s_zk, g))

    def attend(i):
        heads = _ds(i * rep, rep, rep)
        q_i = q_s[heads, :]
        do_i = do_s[heads, :]
        k = k_v[i]
        v = v_v[i]
        s = _dot(q_i, k, NT) * scale
        e = jnp.exp(s - jnp.max(s, axis=-1, keepdims=True))
        p = e / jnp.sum(e, axis=-1, keepdims=True)
        dp = _dot(do_i, v, NT)
        d_sc = p * (dp - jnp.sum(p * dp, axis=-1, keepdims=True)) * scale
        o_s[heads, :] = _dot(p, v, NN)
        dq_s[heads, :] = _dot(d_sc, k, NN)
        stream, group = lax.div(i, n_group), lax.rem(i, n_group)
        dk_v[stream, group] = _dot(d_sc, q_i, TN).astype(BF16)
        dv_v[stream, group] = _dot(p, do_i, TN).astype(BF16)

    def attend_group(g):
        first, half = g * STREAMS, STREAMS // 2
        _loop(first, first + half, attend)
        write_zeros(dv_h, s_zv, g, 0, n_zero // 2)
        _loop(first + half, first + STREAMS, attend)
        write_zeros(dv_h, s_zv, g, n_zero // 2)

    _loop(0, n_group, attend_group)

    def heads_to_rows(ref):
        return jnp.concatenate(
            [ref[pl.ds(h, batch, stride=HQ), :] for h in range(HQ)], axis=1)

    o = heads_to_rows(o_s)
    s_out_proj = _dot(o, _matrix(wo_v), NN)
    out_v[...] = (x + s_out_proj * gate).astype(BF16)
    store(dwo_v, _dot(o, d_s, TN))
    _copy(out_v, out_h, s_out)
    _loop(0, n_group // 2, lambda g: write_window(dk_v, dk_h, s_dk, g))

    dq = heads_to_rows(dq_s)
    store(dwq_v, _dot(xn, dq, TN))
    _loop(n_group // 2, n_group, lambda g: write_window(dk_v, dk_h, s_dk, g))

    d_xn = _dot(dq, _matrix(wq_v), NT)
    d_y = go * s_out_proj * (sig * (1.0 + y * (1.0 - sig)))
    store(dw4_v, _dot(act, d_y, TN))
    _loop(0, n_group // 2, lambda g: write_window(dv_v, dv_h, s_dv, g))

    d_z = _dot(d_y, _matrix(w4_v), NT) * dact
    store(dw3_v, _dot(ln2, d_z, TN))
    d_xn = d_xn + d_y + _layernorm_bwd(_dot(d_z, _matrix(w3_v), NT), ln2, rstd2)
    dx_v[...] = (go + _layernorm_bwd(d_xn, xn, rstd1)).astype(BF16)
    _loop(n_group // 2, n_group, lambda g: write_window(dv_v, dv_h, s_dv, g))
    _copy(dx_v, dx_h, s_dx)

    _loop(0, dwo_v.shape[1] // 32, lambda i: write_rows(dwo_v, dwo_h, s_dwo, i, 32))

    def write_dwq(i):
        split = dw3_v.shape[2]
        write_rows(dwq_v, dwq_h, s_dwq, i, 8, pl.ds(0, split))
        write_rows(dwq_v, dwq_h, s_dwq, i, 8, pl.ds(split, dwq_v.shape[2] - split))

    _loop(0, dwq_v.shape[1] // 8, write_dwq)

    def write_mlp(i):
        write_rows(dw3_v, dw3_h, s_dw3, i, 8)
        write_rows(dw4_v, dw4_h, s_dw4, i, 32)

    n_both = dw4_v.shape[1] // 32
    _loop(0, n_both, write_mlp)
    for i in range(n_both, dw3_v.shape[1] // 8):
        write_rows(dw3_v, dw3_h, s_dw3, i, 8)

    _wait(dk_h.at[:, :, pl.ds(0, front)], s_zk)
    _wait(dv_h.at[:, :, pl.ds(0, front)], s_zv)
    for ref, sem in ((out_v, s_out), (dk_v, s_dk), (dv_v, s_dv), (dx_v, s_dx),
                     (dwo_v, s_dwo), (dwq_v, s_dwq), (dw4_v, s_dw4),
                     (dw3_v, s_dw3)):
        _wait(ref, sem)


@jax.jit
def pallas_recurrent_scan__sliding_block_cached__mixer_s_mlp__decode_kernel(
    A_x: jax.Array,
    A_k_cache: jax.Array,
    A_v_cache: jax.Array,
    A_wq: jax.Array,
    A_wo: jax.Array,
    B_x: jax.Array,
    B_w1: jax.Array,
    B_w2: jax.Array,
    B_w3: jax.Array,
    B_w4: jax.Array,
    grad_out: jax.Array,
):
    del B_x, B_w1, B_w2
    batch, seq, d_model = A_x.shape
    assert seq == 1
    _, n_kv, s_k, d_head = A_k_cache.shape
    win = min(4096, max(256, s_k // 4))
    n_pair = batch * n_kv
    row = (batch, d_model)
    groups = (STREAMS, n_pair // STREAMS)
    weights = tuple(
        (n, w.shape[0] // n, w.shape[1])
        for w, n in ((A_wq, STREAMS), (A_wo, STREAMS),
                     (B_w3, MLP_STREAMS), (B_w4, MLP_STREAMS))
    )
    heads = pltpu.VMEM((batch * HQ, d_head), F32)
    hbm = pl.BlockSpec(memory_space=pltpu.HBM)

    outs = pl.pallas_call(
        _kernel,
        in_specs=[hbm] * 8,
        out_specs=[hbm] * 8,
        out_shape=[
            jax.ShapeDtypeStruct(s, BF16)
            for s in (row, row, *[(*groups, s_k, d_head)] * 2, *weights)
        ],
        scratch_shapes=[
            *[pltpu.VMEM(s, BF16)
              for s in (row, row, *[(n_pair, win, d_head)] * 2, *weights)],
            *[pltpu.VMEM(s, BF16)
              for s in (row, row, *[(*groups, win, d_head)] * 2, *weights)],
            pltpu.VMEM((STREAMS, WRITE_ROWS, d_head), BF16),
            heads, heads, heads, heads,
            pltpu.SemaphoreType.DMA((18,)),
        ],
        compiler_params=pltpu.CompilerParams(
            vmem_limit_bytes=120 * 1024 * 1024,
            disable_bounds_checks=True,
            disable_semaphore_checks=True,
        ),
    )(
        A_x.reshape(row), grad_out.reshape(row),
        A_k_cache.reshape(n_pair, s_k, d_head),
        A_v_cache.reshape(n_pair, s_k, d_head),
        *(w.reshape(s) for w, s in zip((A_wq, A_wo, B_w3, B_w4), weights)),
    )
    return tuple(
        o.reshape(like.shape)
        for o, like in zip(outs, (A_x, A_x, A_k_cache, A_v_cache,
                                  A_wq, A_wo, B_w3, B_w4))
    )
```

```python
import jax
import jax.numpy as jnp
from jax import lax
import jax.experimental.pallas as pl
import jax.experimental.pallas.tpu as pltpu

F32 = jnp.float32
BF16 = jnp.bfloat16

HQ = 32
DH = 128
EPS = 1e-5

STREAMS = 8
READ_ROWS = 16
READ_COLS = 256
WRITE_ROWS = 112

NN = (((1,), (0,)), ((), ()))
NT = (((1,), (1,)), ((), ()))
TN = (((0,), (0,)), ((), ()))


def _dot(a, b, dims):
    return lax.dot_general(
        a.astype(BF16), b.astype(BF16), dims, preferred_element_type=F32
    )


def _layernorm(x):
    xc = x - jnp.mean(x, axis=-1, keepdims=True)
    var = jnp.mean(xc * xc, axis=-1, keepdims=True)
    rstd = 1.0 / jnp.sqrt(var + EPS)
    return xc * rstd, rstd


def _layernorm_bwd(dy, y, rstd):
    return rstd * (
        dy
        - jnp.mean(dy, axis=-1, keepdims=True)
        - y * jnp.mean(dy * y, axis=-1, keepdims=True)
    )


def _gelu_and_grad(z):
    c0, c1 = 0.7978845608028654, 0.044715
    t = jnp.tanh(c0 * (z + c1 * z * z * z))
    cdf = 0.5 * (1.0 + t)
    dcdf = 0.5 * (1.0 - t * t) * c0 * (1.0 + 3.0 * c1 * z * z)
    return z * cdf, cdf + z * dcdf


def _copy(src, dst, sem, priority=0):
    pltpu.make_async_copy(src, dst, sem).start(priority=priority)


def _wait(ref, sem):
    pltpu.make_async_copy(ref, ref, sem).wait()


def _loop(lo, hi, body):
    def step(i, carry):
        body(i)
        return carry

    lax.fori_loop(lo, hi, step, None)


def _ds(start, size, multiple):
    if isinstance(start, int):
        return pl.ds(start, size)
    return pl.ds(pl.multiple_of(start, multiple), size)


def _matrix(ref):
    streams, n_rows, n_cols = ref.shape
    return ref[...].reshape(streams * n_rows, n_cols)


def _kernel(
    x_h, go_h, k_h, v_h, wq_h, wo_h, w3_h, w4_h,
    out_h, dx_h, dk_h, dv_h, dwq_h, dwo_h, dw3_h, dw4_h,
    x_v, go_v, k_v, v_v, wq_v, wo_v, w3_v, w4_v,
    out_v, dx_v, dk_v, dv_v, dwq_v, dwo_v, dw3_v, dw4_v,
    zero_v, q_s, do_s, o_s, dq_s,
    sems,
):
    n_pair, cache_len, _ = k_h.shape
    n_group = dk_h.shape[1]
    win = k_v.shape[1]
    front = cache_len - win
    batch = x_h.shape[0]
    n_kv = n_pair // batch
    rep = HQ // n_kv
    scale = DH**-0.5
    (s_x, s_go, s_k, s_v, s_wq, s_wo, s_w3, s_w4, s_zk, s_zv,
     s_out, s_dx, s_dk, s_dv, s_dwq, s_dwo, s_dw3, s_dw4) = (
        sems.at[i] for i in range(18))

    def read_group(g):
        pairs = pl.ds(g * STREAMS, STREAMS)

        def read_rows(i):
            src = _ds(front + i * READ_ROWS, READ_ROWS, READ_ROWS)
            dst = _ds(i * READ_ROWS, READ_ROWS, READ_ROWS)
            _copy(k_h.at[pairs, src, :], k_v.at[pairs, dst, :], s_k, 0)
            _copy(v_h.at[pairs, src, :], v_v.at[pairs, dst, :], s_v, 1)

        _loop(0, win // READ_ROWS, read_rows)

    _loop(0, n_pair // STREAMS, read_group)

    _copy(x_h, x_v, s_x, 0)
    _copy(go_h, go_v, s_go, 1)

    def read_weights(wide_h, wide_v, wide_sem, tall_h, tall_v, tall_sem):
        per_wide = wide_h.shape[2] // READ_COLS
        per_tall = tall_h.shape[2] // READ_COLS

        def read_rows(i):
            for c in range(per_wide):
                tile = (slice(None), _ds(i * 8, 8, 8),
                        pl.ds(c * READ_COLS, READ_COLS))
                _copy(wide_h.at[tile], wide_v.at[tile], wide_sem, 0)
                j = i * per_wide + c
                tile = (slice(None), _ds(lax.div(j, per_tall) * 8, 8, 8),
                        _ds(lax.rem(j, per_tall) * READ_COLS, READ_COLS, READ_COLS))
                _copy(tall_h.at[tile], tall_v.at[tile], tall_sem, 1)

        _loop(0, wide_h.shape[1] // 8, read_rows)

    read_weights(wq_h, wq_v, s_wq, wo_h, wo_v, s_wo)
    zero_v[...] = jnp.zeros(zero_v.shape, BF16)
    read_weights(w3_h, w3_v, s_w3, w4_h, w4_v, s_w4)
    _wait(w3_v, s_w3)

    n_zero, zero_tail = divmod(front, WRITE_ROWS)
    n_win, win_tail = divmod(win, WRITE_ROWS)

    def write_zeros(dst_h, sem, g, lo=0, hi=n_zero):
        def body(i):
            dst = _ds(i * WRITE_ROWS, WRITE_ROWS, 16)
            _copy(zero_v, dst_h.at[:, g, dst, :], sem)

        _loop(lo, hi, body)
        if hi == n_zero and zero_tail:
            _copy(zero_v.at[:, pl.ds(0, zero_tail), :],
                  dst_h.at[:, g, pl.ds(front - zero_tail, zero_tail), :], sem)

    def write_window(src_v, dst_h, sem, g):
        def body(i):
            src = _ds(i * WRITE_ROWS, WRITE_ROWS, 16)
            dst = _ds(front + i * WRITE_ROWS, WRITE_ROWS, 16)
            _copy(src_v.at[:, g, src, :], dst_h.at[:, g, dst, :], sem)

        _loop(0, n_win, body)
        if win_tail:
            _copy(src_v.at[:, g, pl.ds(win - win_tail, win_tail), :],
                  dst_h.at[:, g, pl.ds(cache_len - win_tail, win_tail), :], sem)

    def write_rows(src_v, dst_h, sem, i, n_rows, cols=slice(None)):
        tile = (slice(None), _ds(i * n_rows, n_rows, n_rows), cols)
        _copy(src_v.at[tile], dst_h.at[tile], sem)

    def store(ref, value):
        ref[...] = value.astype(BF16).reshape(ref.shape)

    write_zeros(dk_h, s_zk, 0)
    for ref, sem in ((x_v, s_x), (go_v, s_go), (w4_v, s_w4), (wq_v, s_wq),
                     (wo_v, s_wo), (k_v, s_k), (v_v, s_v)):
        _wait(ref, sem)
    x = x_v[...].astype(F32)
    go = go_v[...].astype(F32)
    xn, rstd1 = _layernorm(x)
    ln2, rstd2 = _layernorm(xn)
    act, dact = _gelu_and_grad(_dot(ln2, _matrix(w3_v), NN))
    y = xn + _dot(act, _matrix(w4_v), NN)
    sig = jax.nn.sigmoid(y)
    gate = y * sig
    d_s = go * gate
    q = _dot(xn, _matrix(wq_v), NN)
    d_o = _dot(d_s, _matrix(wo_v), NT)
    for h in range(HQ):
        q_s[:, h, :] = q[:, h * DH:(h + 1) * DH]
        do_s[:, h, :] = d_o[:, h * DH:(h + 1) * DH]
    _loop(1, n_group, lambda g: write_zeros(dk_h, s_zk, g))

    def attend(i):
        heads = (lax.div(i, n_kv), _ds(lax.rem(i, n_kv) * rep, rep, rep))
        q_i = q_s[heads]
        do_i = do_s[heads]
        k = k_v[i]
        v = v_v[i]
        s = _dot(q_i, k, NT) * scale
        e = jnp.exp(s - jnp.max(s, axis=-1, keepdims=True))
        p = e / jnp.sum(e, axis=-1, keepdims=True)
        dp = _dot(do_i, v, NT)
        d_sc = p * (dp - jnp.sum(p * dp, axis=-1, keepdims=True)) * scale
        o_s[heads] = _dot(p, v, NN)
        dq_s[heads] = _dot(d_sc, k, NN)
        stream, group = lax.div(i, n_group), lax.rem(i, n_group)
        dk_v[stream, group] = _dot(d_sc, q_i, TN).astype(BF16)
        dv_v[stream, group] = _dot(p, do_i, TN).astype(BF16)

    def attend_group(g):
        first, half = g * STREAMS, STREAMS // 2
        _loop(first, first + half, attend)
        write_zeros(dv_h, s_zv, g, 0, n_zero // 2)
        _loop(first + half, first + STREAMS, attend)
        write_zeros(dv_h, s_zv, g, n_zero // 2)

    _loop(0, n_group, attend_group)

    def heads_to_rows(ref):
        return jnp.concatenate([ref[:, h, :] for h in range(HQ)], axis=1)

    o = heads_to_rows(o_s)
    s_out_proj = _dot(o, _matrix(wo_v), NN)
    out_v[...] = (x + s_out_proj * gate).astype(BF16)
    store(dwo_v, _dot(o, d_s, TN))
    _copy(out_v, out_h, s_out)
    _loop(0, n_group // 2, lambda g: write_window(dk_v, dk_h, s_dk, g))

    dq = heads_to_rows(dq_s)
    store(dwq_v, _dot(xn, dq, TN))
    _loop(n_group // 2, n_group, lambda g: write_window(dk_v, dk_h, s_dk, g))

    d_xn = _dot(dq, _matrix(wq_v), NT)
    d_y = go * s_out_proj * (sig * (1.0 + y * (1.0 - sig)))
    store(dw4_v, _dot(act, d_y, TN))
    _loop(0, n_group // 2, lambda g: write_window(dv_v, dv_h, s_dv, g))

    d_z = _dot(d_y, _matrix(w4_v), NT) * dact
    store(dw3_v, _dot(ln2, d_z, TN))
    d_xn = d_xn + d_y + _layernorm_bwd(_dot(d_z, _matrix(w3_v), NT), ln2, rstd2)
    dx_v[...] = (go + _layernorm_bwd(d_xn, xn, rstd1)).astype(BF16)
    _loop(n_group // 2, n_group, lambda g: write_window(dv_v, dv_h, s_dv, g))
    _copy(dx_v, dx_h, s_dx)

    def write_attn_grads(i):
        left = WRITE_ROWS * DH // 8
        right = dwq_v.shape[2] - left
        write_rows(dwq_v, dwq_h, s_dwq, i, 8, pl.ds(0, left))
        write_rows(dwo_v, dwo_h, s_dwo, 2 * i, 32)
        write_rows(dwq_v, dwq_h, s_dwq, i, 8, pl.ds(left, right))
        write_rows(dwo_v, dwo_h, s_dwo, 2 * i + 1, 32)

    _loop(0, dwq_v.shape[1] // 8, write_attn_grads)

    def write_mlp_grads(i):
        write_rows(dw3_v, dw3_h, s_dw3, i, 8)
        write_rows(dw4_v, dw4_h, s_dw4, i, 32)

    n_both = dw4_v.shape[1] // 32
    _loop(0, n_both, write_mlp_grads)
    for i in range(n_both, dw3_v.shape[1] // 8):
        write_rows(dw3_v, dw3_h, s_dw3, i, 8)

    _wait(dk_h.at[:, :, pl.ds(0, front)], s_zk)
    _wait(dv_h.at[:, :, pl.ds(0, front)], s_zv)
    for ref, sem in ((out_v, s_out), (dk_v, s_dk), (dv_v, s_dv), (dx_v, s_dx),
                     (dwo_v, s_dwo), (dwq_v, s_dwq), (dw4_v, s_dw4),
                     (dw3_v, s_dw3)):
        _wait(ref, sem)


@jax.jit
def pallas_recurrent_scan__sliding_block_cached__mixer_s_mlp__decode_kernel(
    A_x: jax.Array,
    A_k_cache: jax.Array,
    A_v_cache: jax.Array,
    A_wq: jax.Array,
    A_wo: jax.Array,
    B_x: jax.Array,
    B_w1: jax.Array,
    B_w2: jax.Array,
    B_w3: jax.Array,
    B_w4: jax.Array,
    grad_out: jax.Array,
):
    del B_x, B_w1, B_w2
    batch, seq, d_model = A_x.shape
    assert seq == 1
    _, n_kv, s_k, d_head = A_k_cache.shape
    win = min(4096, max(256, s_k // 4))
    n_pair = batch * n_kv
    row = (batch, d_model)
    groups = (STREAMS, n_pair // STREAMS)

    def split(w, streams):
        return (streams, w.shape[0] // streams, w.shape[1])

    weights = (split(A_wq, STREAMS), split(A_wo, STREAMS),
               split(B_w3, STREAMS // 2), split(B_w4, STREAMS // 2))
    grads = tuple(split(w, STREAMS // 2) for w in (A_wq, A_wo, B_w3, B_w4))
    heads = pltpu.VMEM((batch, HQ, d_head), F32)
    hbm = pl.BlockSpec(memory_space=pltpu.HBM)

    outs = pl.pallas_call(
        _kernel,
        in_specs=[hbm] * 8,
        out_specs=[hbm] * 8,
        out_shape=[
            jax.ShapeDtypeStruct(s, BF16)
            for s in (row, row, *[(*groups, s_k, d_head)] * 2, *grads)
        ],
        scratch_shapes=[
            *[pltpu.VMEM(s, BF16)
              for s in (row, row, *[(n_pair, win, d_head)] * 2, *weights)],
            *[pltpu.VMEM(s, BF16)
              for s in (row, row, *[(*groups, win, d_head)] * 2, *grads)],
            pltpu.VMEM((STREAMS, WRITE_ROWS, d_head), BF16),
            heads, heads, heads, heads,
            pltpu.SemaphoreType.DMA((18,)),
        ],
        compiler_params=pltpu.CompilerParams(
            vmem_limit_bytes=120 * 1024 * 1024,
            disable_bounds_checks=True,
            disable_semaphore_checks=True,
        ),
    )(
        A_x.reshape(row), grad_out.reshape(row),
        A_k_cache.reshape(n_pair, s_k, d_head),
        A_v_cache.reshape(n_pair, s_k, d_head),
        *(w.reshape(s) for w, s in zip((A_wq, A_wo, B_w3, B_w4), weights)),
    )
    return tuple(
        o.reshape(like.shape)
        for o, like in zip(outs, (A_x, A_x, A_k_cache, A_v_cache,
                                  A_wq, A_wo, B_w3, B_w4))
    )
```
